```python
import jax
import jax.numpy as jnp

def _softmax(x, axis=-1):
    return jax.nn.softmax(x, axis=axis)
def _gelu(x):
    return jax.nn.gelu(x, approximate=True)
def _silu(x):
    return jax.nn.silu(x)
def _sigmoid(x):
    return jax.nn.sigmoid(x)
def _layernorm(x, axis=-1, eps=1e-5):
    m = jnp.mean(x, axis=axis, keepdims=True)
    v = jnp.var(x, axis=axis, keepdims=True)
    return (x - m) / jnp.sqrt(v + eps)
def _scatter_add(tgt, idx, src, axis=0):
    return tgt.at[idx].add(src)
def _segment_sum(src, seg, n):
    return jax.ops.segment_sum(src, seg, n)
class _Rng:
    def __init__(self, key):
        self._k = key
    def _next(self):
        self._k, sub = jax.random.split(self._k)
        return sub
    def normal(self, shape):
        return jax.random.normal(self._next(), shape, dtype=jnp.bfloat16)
    def randint(self, lo, hi, shape):
        return jax.random.randint(self._next(), shape, lo, hi, dtype=jnp.int32)
    def uniform(self, shape, lo=0.0, hi=1.0):
        return jax.random.uniform(self._next(), shape, jnp.bfloat16, lo, hi)
    def permutation(self, n):
        return jax.random.permutation(self._next(), n)


kernel_name = 'standalone__instancenorm__prompt'

def setup_inputs():
    _rng = _Rng(jax.random.key(int.from_bytes(__import__("os").urandom(4), "little")))
    _w = (lambda a: (lambda t: t.astype(jnp.bfloat16) if jnp.issubdtype(t.dtype, jnp.floating) else t)(jnp.asarray(a)))
    B, C, H, W = 2, 1024, 2048, 32
    return {
        "x": _w((lambda *s: _rng.normal(s) * 0.05)(B, C, H, W)),
        "g": _w((lambda *s: _rng.normal(s) * 0.05)(C) + 1.0),
        "b": _w((lambda *s: _rng.normal(s) * 0.05)(C)),
    }

def reference(x, g, b):
    mu = x.mean(axis=(-2, -1), keepdims=True)
    var = ((x - mu) * (x - mu)).mean(axis=(-2, -1), keepdims=True)
    xhat = (x - mu) / jnp.sqrt(var + 1e-5)
    return xhat * g.reshape(1, -1, 1, 1) + b.reshape(1, -1, 1, 1)
```

```python
import jax
import jax.numpy as jnp
import jax.experimental.pallas as pl
import jax.experimental.pallas.tpu as pltpu

EPS = 1e-5
LANES = 128
UNIT_ROWS = 128
PIECES = 32
INST_PER_UNIT = 8
GA = 64
LOOKAHEAD = 4
RS = 4
WNA = 8
TAIL = 2
EARLY_W = 2


def _tree_sum(xs):
    xs = list(xs)
    while len(xs) > 1:
        nxt = [xs[i] + xs[i + 1] for i in range(0, len(xs) - 1, 2)]
        if len(xs) % 2:
            nxt.append(xs[-1])
        xs = nxt
    return xs[0]


def _full_sum(acc):
    return jnp.sum(jnp.sum(acc, axis=0, keepdims=True), axis=1, keepdims=True)


def _normalize_unit(buf, a, ch0, g_ref, b_ref, inv_n):
    def ld(j, q):
        v = buf[a, 4 * j + q // 2, pl.ds((q % 2) * 64, 64), :]
        return v.astype(jnp.float32).reshape(8, 8, LANES)

    mus = []
    for j in range(INST_PER_UNIT):
        acc = _tree_sum([jnp.sum(ld(j, q), axis=0) for q in range(8)])
        mus.append(_full_sum(acc) * inv_n)
    scs = []
    for j in range(INST_PER_UNIT):
        parts = []
        for q in range(8):
            d = ld(j, q) - mus[j]
            parts.append(jnp.sum(d * d, axis=0))
        var = _full_sum(_tree_sum(parts)) * inv_n
        scs.append(jax.lax.rsqrt(var + EPS) * g_ref[ch0 + j])
    for j in range(INST_PER_UNIT):
        sh = b_ref[ch0 + j] - mus[j] * scs[j]
        for q in range(8):
            y = ld(j, q) * scs[j] + sh
            buf[a, 4 * j + q // 2, pl.ds((q % 2) * 64, 64), :] = (
                y.reshape(64, LANES).astype(buf.dtype))


@jax.jit
def pallas_standalone__instancenorm__prompt_kernel(
    x: jax.Array,
    g: jax.Array,
    b: jax.Array,
):
    B, C, H, W = x.shape
    n_inst = B * C
    assert (H * W) == 4 * UNIT_ROWS * LANES and W % 8 == 0 and H % LANES == 0
    NA = n_inst // INST_PER_UNIT
    ngroups = NA // GA
    nspan = GA // WNA
    RB = PIECES // RS
    inv_n = 1.0 / (H * W)

    def kernel(x_hbm, g_ref, b_ref, o_hbm, buf, rsem, wsem, tsem):
        def read_start(gi, a):
            for s in range(RS):
                pltpu.make_async_copy(
                    x_hbm.at[gi * GA + a, pl.ds(s * RB, RB)],
                    buf.at[a, pl.ds(s * RB, RB)], rsem.at[a]).start()

        def read_wait(a):
            pltpu.make_async_copy(buf.at[a], buf.at[a], rsem.at[a]).wait()

        def write_range(gi, sp, b0, b1, sem):
            for p in range(b0, b1):
                pltpu.make_async_copy(
                    buf.at[pl.ds(sp * WNA, WNA), p],
                    o_hbm.at[pl.ds(gi * GA + sp * WNA, WNA), p], sem).start()

        def write_wait(sp, b0, b1, sem):
            v = buf.at[pl.ds(sp * WNA, WNA), pl.ds(b0, b1 - b0)]
            pltpu.make_async_copy(v, v, sem).wait()

        for a in range(LOOKAHEAD):
            read_start(0, a)

        def group(gi, carry):
            def step(a, c):
                @pl.when(a + LOOKAHEAD < GA)
                def _():
                    read_start(gi, a + LOOKAHEAD)

                read_wait(a)

                @pl.when(a == GA - 1)
                def _():
                    write_range(gi, 0, EARLY_W, PIECES, wsem.at[0])

                    def wsp(sp, c2):
                        write_range(gi, sp, 0, PIECES, wsem.at[sp])
                        return c2

                    jax.lax.fori_loop(1, nspan - 1, wsp, 0)

                ch0 = ((gi * GA + a) * INST_PER_UNIT) % C
                _normalize_unit(buf, a, ch0, g_ref, b_ref, inv_n)

                @pl.when(a == GA - 2)
                def _():
                    write_range(gi, 0, 0, EARLY_W, wsem.at[0])

                return c

            jax.lax.fori_loop(0, GA, step, 0)
            write_range(gi, nspan - 1, 0, PIECES - TAIL, wsem.at[nspan - 1])
            write_range(gi, nspan - 1, PIECES - TAIL, PIECES, tsem)
            for sp in range(nspan - 1):
                write_wait(sp, 0, PIECES, wsem.at[sp])
            write_wait(nspan - 1, 0, PIECES - TAIL, wsem.at[nspan - 1])

            @pl.when(gi + 1 < ngroups)
            def _():
                for a in range(LOOKAHEAD):
                    read_start(gi + 1, a)

            write_wait(nspan - 1, PIECES - TAIL, PIECES, tsem)
            return carry

        jax.lax.fori_loop(0, ngroups, group, 0)

    xt = x.transpose(0, 1, 3, 2).reshape(n_inst, W // 8, 8, H // LANES, LANES)
    xt = xt.transpose(0, 1, 3, 2, 4).reshape(NA, PIECES, UNIT_ROWS, LANES)
    y = pl.pallas_call(
        kernel,
        in_specs=[
            pl.BlockSpec(memory_space=pl.ANY),
            pl.BlockSpec(memory_space=pltpu.SMEM),
            pl.BlockSpec(memory_space=pltpu.SMEM),
        ],
        out_specs=pl.BlockSpec(memory_space=pl.ANY),
        out_shape=jax.ShapeDtypeStruct((NA, PIECES, UNIT_ROWS, LANES), x.dtype),
        scratch_shapes=[
            pltpu.VMEM((GA, PIECES, UNIT_ROWS, LANES), x.dtype),
            pltpu.SemaphoreType.DMA((GA,)),
            pltpu.SemaphoreType.DMA((nspan,)),
            pltpu.SemaphoreType.DMA(()),
        ],
        compiler_params=pltpu.CompilerParams(
            vmem_limit_bytes=(GA + 8) * 1024 * 1024),
    )(xt, g.astype(jnp.float32), b.astype(jnp.float32))
    y = y.reshape(n_inst, W // 8, H // LANES, 8, LANES).transpose(0, 1, 3, 2, 4)
    return y.reshape(B, C, W, H).transpose(0, 1, 3, 2)
```

```python
import jax
import jax.numpy as jnp
import jax.experimental.pallas as pl
import jax.experimental.pallas.tpu as pltpu

EPS = 1e-5
LANES = 128
ROWS = 64
NQ = 8
NJ = 8
SPAN = 8
GA = 96
LOOKAHEAD = 8
NSEM = 16
EARLY_W = 8
EARLY_AT = 4
LAG = 7
NWP = NJ * NQ // 2


def _tree_sum(xs):
    xs = list(xs)
    while len(xs) > 1:
        nxt = [xs[i] + xs[i + 1] for i in range(0, len(xs) - 1, 2)]
        if len(xs) % 2:
            nxt.append(xs[-1])
        xs = nxt
    return xs[0]


def _full_sum_bcast(acc):
    s = jnp.sum(jnp.sum(acc, axis=0, keepdims=True), axis=1, keepdims=True)
    return jnp.broadcast_to(s, acc.shape)


@jax.jit
def pallas_standalone__instancenorm__prompt_kernel(
    x: jax.Array,
    g: jax.Array,
    b: jax.Array,
):
    B, C, H, W = x.shape
    n_inst = B * C
    assert H * W == NQ * ROWS * LANES and W % 8 == 0 and H % LANES == 0
    assert C & (C - 1) == 0 and n_inst % (NJ * SPAN) == 0
    NA = n_inst // NJ
    ngroups = -(-NA // GA)
    last_rows = NA - (ngroups - 1) * GA
    assert GA % SPAN == 0 and last_rows % SPAN == 0 and last_rows >= 4 * SPAN
    assert EARLY_AT < LOOKAHEAD < NSEM
    DUMMY = GA * NJ
    inv_n = 1.0 / (H * W)
    f32 = jnp.float32

    def kernel(x_hbm, g_hbm, b_hbm, o_hbm, buf, g_s, b_s, rsem, wsem, tsem, psem):
        def read_desc(base, k, r0, nr):
            a0 = ((k >> 6) << 3) + r0
            j = (k >> 3) & 7
            q = k & 7
            return pltpu.make_async_copy(
                x_hbm.at[pl.ds(base + a0, nr), j, q],
                buf.at[pl.ds(a0, nr), j, q],
                rsem.at[k & (NSEM - 1)])

        def read_start(base, k):
            read_desc(base, k, 0, SPAN - 1).start(priority=1)
            read_desc(base, k, SPAN - 1, 1).start(priority=0)

        def read_wait(base, k):
            read_desc(base, k, 0, SPAN).wait()

        def write_desc(base, sp, idx, sem):
            return pltpu.make_async_copy(
                buf.at[(pl.ds(sp * SPAN, SPAN),) + idx],
                o_hbm.at[(pl.ds(base + sp * SPAN, SPAN),) + idx], sem)

        def write_range(base, sp, p0, p1, sem):
            for p in range(p0, p1):
                write_desc(base, sp, (p // 4, pl.ds(2 * (p % 4), 2)), sem).start()

        def first_reads(base):
            for k in range(LOOKAHEAD):
                read_start(base, k)

        def loc(m, M):
            valid = jnp.logical_and(m >= 0, m < M)
            i = (m & ~63) + ((m & 7) << 3) + ((m >> 3) & 7)
            return jnp.where(valid, i, DUMMY)

        def ld(i, q):
            return buf[i >> 3, i & 7, q].astype(f32).reshape(ROWS // 8, 8, LANES)

        def stages(base, M, k, carry, start_next=None):
            acc1, mu_a, mu_b, mu_c, acc2, sc, sh, locs = carry
            i1, _, i2, ir, i3 = locs
            new_acc1 = _tree_sum([jnp.sum(ld(i1, q), axis=0) for q in range(NQ)])
            if start_next is not None:
                start_next()
            parts = []
            for q in range(NQ):
                d = ld(i2, q) - mu_a
                parts.append(jnp.sum(d * d, axis=0))
            new_acc2 = _tree_sum(parts)
            new_mu = _full_sum_bcast(acc1) * inv_n
            ch = (base * NJ + ir) & (C - 1)
            var = _full_sum_bcast(acc2) * inv_n
            new_sc = jax.lax.rsqrt(var + EPS) * g_s[ch].astype(f32)
            new_sh = jnp.full((8, LANES), b_s[ch].astype(f32), f32)
            for q in range(NQ):
                y = (ld(i3, q) - mu_c) * sc + sh
                buf[i3 >> 3, i3 & 7, q] = y.reshape(ROWS, LANES).astype(buf.dtype)
            new_locs = (loc(k + 1 - LAG, M),) + locs[:-1]
            return (new_acc1, new_mu, mu_a, mu_b, new_acc2, new_sc, new_sh, new_locs)

        first_reads(0)
        cg = pltpu.make_async_copy(g_hbm, g_s, psem.at[0])
        cb = pltpu.make_async_copy(b_hbm, b_s, psem.at[1])
        cg.start()
        cb.start()
        buf[GA, 0] = jnp.zeros((NQ, ROWS, LANES), buf.dtype)
        cg.wait()
        cb.wait()

        def group(gi, carry0):
            base = gi * GA
            rows = jnp.minimum(GA, NA - base)
            M = rows * NJ
            nspan = rows >> 3

            def step_main(k, carry):
                read_wait(base, k)
                return stages(base, M, k, carry,
                              lambda: read_start(base, k + LOOKAHEAD))

            def step_tail(k, carry):
                @pl.when(k < M)
                def _():
                    read_wait(base, k)

                @pl.when(k == M - 1 - EARLY_AT)
                def _():
                    write_range(base, 0, 0, EARLY_W, wsem.at[0])

                @pl.when(k == M - 1)
                def _():
                    write_range(base, 0, EARLY_W, NWP, wsem.at[0])
                    write_range(base, 1, 0, NWP, wsem.at[1])

                return stages(base, M, k, carry)

            z = jnp.zeros((8, LANES), f32)
            carry = (z,) * 7 + ((jnp.int32(DUMMY),) * 5,)
            carry = jax.lax.fori_loop(0, M - LOOKAHEAD, step_main, carry)
            jax.lax.fori_loop(M - LOOKAHEAD, M + LAG + 4, step_tail, carry)

            def start_span(sp, c):
                write_range(base, sp, 0, NWP, wsem.at[sp])
                return c

            def wait_span(sp, c):
                write_desc(base, sp, (), wsem.at[sp]).wait()
                return c

            last = nspan - 1
            jax.lax.fori_loop(2, last, start_span, 0)
            write_range(base, last, 0, NWP - 4, wsem.at[last])
            write_range(base, last, NWP - 4, NWP - 1, tsem.at[0])
            write_range(base, last, NWP - 1, NWP, tsem.at[1])
            jax.lax.fori_loop(0, last, wait_span, 0)
            write_desc(base, last, (pl.ds(0, NJ - 1),), wsem.at[last]).wait()
            write_desc(base, last, (NJ - 1, pl.ds(0, NQ - 2)), tsem.at[0]).wait()

            @pl.when(gi + 1 < ngroups)
            def _():
                first_reads(base + GA)

            write_desc(base, last, (NJ - 1, pl.ds(NQ - 2, 2)), tsem.at[1]).wait()
            return carry0

        jax.lax.fori_loop(0, ngroups, group, 0)

    view = (NA, NJ, NQ, ROWS, LANES)
    xt = x.transpose(0, 1, 3, 2).reshape(n_inst, W // 8, 8, H // LANES, LANES)
    xt = xt.transpose(0, 1, 3, 2, 4).reshape(view)
    y = pl.pallas_call(
        kernel,
        in_specs=[pl.BlockSpec(memory_space=pl.ANY)] * 3,
        out_specs=pl.BlockSpec(memory_space=pl.ANY),
        out_shape=jax.ShapeDtypeStruct(view, x.dtype),
        scratch_shapes=[
            pltpu.VMEM((GA + 1,) + view[1:], x.dtype),
            pltpu.SMEM((C,), g.dtype),
            pltpu.SMEM((C,), b.dtype),
            pltpu.SemaphoreType.DMA((NSEM,)),
            pltpu.SemaphoreType.DMA((GA // SPAN,)),
            pltpu.SemaphoreType.DMA((2,)),
            pltpu.SemaphoreType.DMA((2,)),
        ],
        compiler_params=pltpu.CompilerParams(
            vmem_limit_bytes=(GA + 4) * 1024 * 1024,
            disable_bounds_checks=True),
    )(xt, g, b)
    y = y.reshape(n_inst, W // 8, H // LANES, 8, LANES).transpose(0, 1, 3, 2, 4)
    return y.reshape(B, C, W, H).transpose(0, 1, 3, 2)
```

```python
import jax
import jax.numpy as jnp
import jax.experimental.pallas as pl
import jax.experimental.pallas.tpu as pltpu

EPS = 1e-5
LANES = 128
INST = 512
NJ = 8
NR = 8
ROW = NJ * INST
PIECE = 128
NP = ROW // PIECE
SLAB = 64
GS = 12
SPANS_MAIN = (6, 6)
SPANS_LAST = (8,)
DEPTH = 8
SHIFT = 104
LO_ROWS = (1, 4)
HI_ROWS = (0, 7)
LAG = 9
EARLY_AT = 4
N_EARLY = 8
N_MID = 24
WUNROLL = 8


def _tree_sum(xs):
    xs = list(xs)
    while len(xs) > 1:
        nxt = [xs[i] + xs[i + 1] for i in range(0, len(xs) - 1, 2)]
        if len(xs) % 2:
            nxt.append(xs[-1])
        xs = nxt
    return xs[0]


def _full_sum_bcast(acc):
    s = jnp.sum(jnp.sum(acc, axis=0, keepdims=True), axis=1, keepdims=True)
    return jnp.broadcast_to(s, acc.shape)


@jax.jit
def pallas_standalone__instancenorm__prompt_kernel(
    x: jax.Array,
    g: jax.Array,
    b: jax.Array,
):
    B, C, H, W = x.shape
    n_inst = B * C
    per_super = NR * NJ
    assert H * W == INST * LANES and W % 8 == 0 and H % LANES == 0
    assert C & (C - 1) == 0 and n_inst % per_super == 0
    NS = n_inst // per_super
    ngroups = -(-NS // GS)
    assert sum(SPANS_MAIN) == GS and len(SPANS_MAIN) >= 2
    assert sum(SPANS_LAST) == NS - (ngroups - 1) * GS
    assert N_EARLY * PIECE <= INST * (NJ + (-EARLY_AT - LAG - 5) // NR)
    assert N_MID * PIECE <= INST * (NJ + (-LAG - 5) // NR) and N_MID % WUNROLL == 0
    DUMMY = GS * per_super
    NU = NR * NP
    inv_n = 1.0 / (H * W)
    f32 = jnp.float32

    def kernel(x_hbm, g_hbm, b_hbm, o_hbm, buf, g_s, b_s, rsem, wsem):
        def rd(base, k, rows, off, size):
            s = k >> 6
            return pltpu.make_async_copy(
                x_hbm.at[base + s, rows, pl.ds(off, size)],
                buf.at[s, rows, pl.ds(off, size)],
                rsem.at[k & (DEPTH - 1)])

        def read_start(base, k, static=False):
            p = (k >> 1) & (NP - 1)
            h = k & 1

            def regular():
                off = pl.multiple_of(p * PIECE + (SHIFT - PIECE), 8)
                lo = LO_ROWS[0] + h * (LO_ROWS[1] - LO_ROWS[0])
                hi = HI_ROWS[0] + h * (HI_ROWS[1] - HI_ROWS[0])
                rd(base, k, pl.ds(lo, 3), off, PIECE).start(priority=1)
                rd(base, k, pl.ds(hi, 1), off, PIECE).start(priority=0)

            def ends():
                rows = pl.ds(4 * h, 4)
                rd(base, k, rows, 0, SHIFT).start(priority=1)
                rd(base, k, rows, ROW - PIECE + SHIFT, PIECE - SHIFT).start(priority=0)

            if static:
                (ends if p == 0 else regular)()
            else:
                pl.when(p != 0)(regular)
                pl.when(p == 0)(ends)

        def read_wait(base, k):
            rd(base, k, pl.ds(0, 4), 0, PIECE).wait()

        def first_reads(base):
            for k in range(DEPTH):
                read_start(base, k, static=True)

        def wr(base, s0, na, idx, sem):
            return pltpu.make_async_copy(
                buf.at[(pl.ds(s0, na),) + idx],
                o_hbm.at[(pl.ds(base + s0, na),) + idx], sem)

        def write_start(base, s0, na, u0, u1, sem):
            for u in range(u0, u1):
                wr(base, s0, na, (u // NP, pl.ds((u % NP) * PIECE, PIECE)), sem).start()

        def write_loop(base, s0, na, u0, u1, sem):
            def body(t, c):
                u = t * WUNROLL
                off = pl.multiple_of((u & (NP - 1)) * PIECE, PIECE * WUNROLL)
                for i in range(WUNROLL):
                    wr(base, s0, na, (u >> 5, pl.ds(off + i * PIECE, PIECE)), sem).start()
                return c

            jax.lax.fori_loop(u0 // WUNROLL, u1 // WUNROLL, body, 0)

        def loc(m, M):
            valid = jnp.logical_and(m >= 0, m < M)
            i = (m & ~63) + ((m & 7) << 3) + ((m >> 3) & 7)
            return jnp.where(valid, i, DUMMY)

        def inst(i):
            start = pl.multiple_of((i & 7) * INST, INST)
            return buf.at[i >> 6, (i >> 3) & 7, pl.ds(start, INST)]

        def ld(v, q):
            return v[pl.ds(SLAB * q, SLAB), :].astype(f32).reshape(SLAB // 8, 8, LANES)

        def stages(base, M, k, carry, start_next=None):
            acc1, mu_a, mu_b, mu_c, acc2, sc, sh, locs = carry
            i1, _, i2, ir, i3 = locs
            v1, v2, v3 = inst(i1), inst(i2), inst(i3)
            nq = INST // SLAB
            new_acc1 = _tree_sum([jnp.sum(ld(v1, q), axis=0) for q in range(nq)])
            if start_next is not None:
                start_next()
            parts = []
            for q in range(nq):
                d = ld(v2, q) - mu_a
                parts.append(jnp.sum(d * d, axis=0))
            new_acc2 = _tree_sum(parts)
            new_mu = _full_sum_bcast(acc1) * inv_n
            ch = (base * per_super + ir) & (C - 1)
            var = _full_sum_bcast(acc2) * inv_n
            new_sc = jax.lax.rsqrt(var + EPS) * g_s[ch].astype(f32)
            new_sh = jnp.full((8, LANES), b_s[ch].astype(f32), f32)
            for q in range(nq):
                y = (ld(v3, q) - mu_c) * sc + sh
                v3[pl.ds(SLAB * q, SLAB), :] = y.reshape(SLAB, LANES).astype(buf.dtype)
            new_locs = (loc(k + 1 - LAG, M),) + locs[:-1]
            return (new_acc1, new_mu, mu_a, mu_b, new_acc2, new_sc, new_sh, new_locs)

        first_reads(0)
        cg = pltpu.make_async_copy(g_hbm, g_s, wsem.at[0])
        cb = pltpu.make_async_copy(b_hbm, b_s, wsem.at[1])
        cg.start()
        cb.start()
        buf[GS, 0, pl.ds(0, INST), :] = jnp.zeros((INST, LANES), buf.dtype)
        cg.wait()
        cb.wait()

        def group(gi, carry0):
            base = gi * GS
            M = jnp.minimum(GS, NS - base) * per_super
            is_last = gi == ngroups - 1

            def per_variant(fn):
                pl.when(jnp.logical_not(is_last))(lambda: fn(SPANS_MAIN, False))
                pl.when(is_last)(lambda: fn(SPANS_LAST, True))

            def step_main(k, carry):
                read_wait(base, k)
                return stages(base, M, k, carry, lambda: read_start(base, k + DEPTH))

            def step_tail(k, carry):
                @pl.when(k < M)
                def _():
                    read_wait(base, k)

                @pl.when(k == M - 1 - EARLY_AT)
                def _():
                    per_variant(lambda sp, _: write_start(
                        base, 0, sp[0], 0, N_EARLY, wsem.at[0]))

                @pl.when(k == M - 1)
                def _():
                    per_variant(lambda sp, _: write_start(
                        base, 0, sp[0], N_EARLY, N_MID, wsem.at[0]))

                return stages(base, M, k, carry)

            z = jnp.zeros((8, LANES), f32)
            carry = (z,) * 7 + ((jnp.int32(DUMMY),) * 5,)
            carry = jax.lax.fori_loop(0, M - DEPTH, step_main, carry)
            jax.lax.fori_loop(M - DEPTH, M + LAG + 4, step_tail, carry)

            def write_phase(spans, last):
                geo = [(sum(spans[:i]), na) for i, na in enumerate(spans)]
                for si, (s0, na) in enumerate(geo):
                    u0 = N_MID if si == 0 else 0
                    u1 = NU if (last or si < len(geo) - 1) else NU - WUNROLL
                    write_loop(base, s0, na, u0, u1, wsem.at[0])
                if last:
                    for s0, na in geo:
                        wr(base, s0, na, (), wsem.at[0]).wait()
                    return
                s0, na = geo[-1]
                write_start(base, s0, na, NU - WUNROLL, NU - 1, wsem.at[0])
                write_start(base, s0, na, NU - 1, NU, wsem.at[1])
                for s1, n1 in geo[:-1]:
                    wr(base, s1, n1, (), wsem.at[0]).wait()
                wr(base, s0, na, (pl.ds(0, NR - 1),), wsem.at[0]).wait()
                wr(base, s0, na, (NR - 1, pl.ds(0, ROW - PIECE)), wsem.at[0]).wait()
                first_reads(base + GS)
                wr(base, s0, na, (NR - 1, pl.ds(ROW - PIECE, PIECE)), wsem.at[1]).wait()

            per_variant(write_phase)
            return carry0

        jax.lax.fori_loop(0, ngroups, group, 0)

    view = (NS, NR, ROW, LANES)
    xt = x.transpose(0, 1, 3, 2).reshape(n_inst, W // 8, 8, H // LANES, LANES)
    xt = xt.transpose(0, 1, 3, 2, 4).reshape(view)
    y = pl.pallas_call(
        kernel,
        in_specs=[pl.BlockSpec(memory_space=pl.ANY)] * 3,
        out_specs=pl.BlockSpec(memory_space=pl.ANY),
        out_shape=jax.ShapeDtypeStruct(view, x.dtype),
        scratch_shapes=[
            pltpu.VMEM((GS + 1,) + view[1:], x.dtype),
            pltpu.SMEM((C,), g.dtype),
            pltpu.SMEM((C,), b.dtype),
            pltpu.SemaphoreType.DMA((DEPTH,)),
            pltpu.SemaphoreType.DMA((2,)),
        ],
        compiler_params=pltpu.CompilerParams(
            vmem_limit_bytes=((GS + 1) * 8 + 4) * 1024 * 1024,
            disable_bounds_checks=True),
    )(xt, g, b)
    y = y.reshape(n_inst, W // 8, H // LANES, 8, LANES).transpose(0, 1, 3, 2, 4)
    return y.reshape(B, C, W, H).transpose(0, 1, 3, 2)
```

```python
import jax
import jax.numpy as jnp
import jax.experimental.pallas as pl
import jax.experimental.pallas.tpu as pltpu

EPS = 1e-5
LANES = 128
INST = 512
NJ = 8
NA, NH = 4, 2
ROW = NJ * INST
PIECE = 128
NP = ROW // PIECE
SLAB = 64
GS = 16
SPANS = (8, 8)
DEPTH = 8
SHIFT = 104
LO_ROW = (0, 1)
HI_ROW = (3, 0)
LAG = 9
EARLY_AT = 4
N_EARLY = 8
N_MID = 32
WUNROLL = 8


def _tree_sum(xs):
    xs = list(xs)
    while len(xs) > 1:
        nxt = [xs[i] + xs[i + 1] for i in range(0, len(xs) - 1, 2)]
        if len(xs) % 2:
            nxt.append(xs[-1])
        xs = nxt
    return xs[0]


def _full_sum_bcast(acc):
    s = jnp.sum(jnp.sum(acc, axis=0, keepdims=True), axis=1, keepdims=True)
    return jnp.broadcast_to(s, acc.shape)


@jax.jit
def pallas_standalone__instancenorm__prompt_kernel(
    x: jax.Array,
    g: jax.Array,
    b: jax.Array,
):
    B, C, H, W = x.shape
    n_inst = B * C
    per_super = NA * NH * NJ
    assert H * W == INST * LANES and W % 8 == 0 and H % LANES == 0
    assert C & (C - 1) == 0 and n_inst % (GS * per_super) == 0
    NS = n_inst // per_super
    ngroups = NS // GS
    M = GS * per_super
    assert sum(SPANS) == GS and len(SPANS) >= 2 and N_MID % WUNROLL == 0
    spans = [(sum(SPANS[:i]), n) for i, n in enumerate(SPANS)]
    NU = NA * NH * NP
    inv_n = 1.0 / (H * W)
    f32 = jnp.float32

    def kernel(x_hbm, g_hbm, b_hbm, o_hbm, buf, g_s, b_s, rsem, wsem):
        def rd(base, k, rows, off, size):
            s, h = k >> 6, k & 1
            return pltpu.make_async_copy(
                x_hbm.at[base + s, rows, h, pl.ds(off, size)],
                buf.at[s, rows, h, pl.ds(off, size)],
                rsem.at[k & (DEPTH - 1)])

        def read_start(base, k, kind=None):
            p = (k >> 1) & (NP - 1)
            h = k & 1

            def regular():
                off = pl.multiple_of(p * PIECE + (SHIFT - PIECE), 8)
                lo = LO_ROW[0] + h * (LO_ROW[1] - LO_ROW[0])
                hi = HI_ROW[0] + h * (HI_ROW[1] - HI_ROW[0])
                rd(base, k, pl.ds(lo, NA - 1), off, PIECE).start(priority=1)
                rd(base, k, pl.ds(hi, 1), off, PIECE).start(priority=0)

            def ends():
                rows = pl.ds(0, NA)
                rd(base, k, rows, 0, SHIFT).start(priority=1)
                rd(base, k, rows, ROW - PIECE + SHIFT, PIECE - SHIFT).start(priority=0)

            if kind == "static":
                (ends if p == 0 else regular)()
            elif kind == "regular":
                regular()
            else:
                pl.when(p != 0)(regular)
                pl.when(p == 0)(ends)

        def read_wait(base, k):
            rd(base, k, pl.ds(0, NA), 0, PIECE).wait()

        def first_reads(base):
            for k in range(DEPTH):
                read_start(base, k, "static")

        def wr(base, span, idx, sem):
            s0, n = span
            return pltpu.make_async_copy(
                buf.at[(pl.ds(s0, n),) + idx],
                o_hbm.at[(pl.ds(base + s0, n),) + idx], sem)

        def write_start(base, span, u0, u1, sem):
            for u in range(u0, u1):
                r = u // NP
                idx = (r // NH, r % NH, pl.ds((u % NP) * PIECE, PIECE))
                wr(base, span, idx, sem).start()

        def write_loop(base, span, u0, u1, sem):
            def body(t, c):
                u = t * WUNROLL
                r = u >> 5
                off = pl.multiple_of((u & (NP - 1)) * PIECE, PIECE * WUNROLL)
                for i in range(WUNROLL):
                    idx = (r >> 1, r & 1, pl.ds(off + i * PIECE, PIECE))
                    wr(base, span, idx, sem).start()
                return c

            jax.lax.fori_loop(u0 // WUNROLL, u1 // WUNROLL, body, 0)

        def loc(m):
            m = jnp.minimum(m, M - 1)
            return (m & ~63) + ((m & 7) << 3) + ((m >> 3) & 7)

        def inst(i):
            start = pl.multiple_of((i & 7) * INST, INST)
            return buf.at[i >> 6, (i >> 4) & 3, (i >> 3) & 1, pl.ds(start, INST)]

        def ld(v, q):
            return v[pl.ds(SLAB * q, SLAB), :].astype(f32).reshape(SLAB // 8, 8, LANES)

        def stages(base, k, carry, start_next=None, normalise=True):
            acc1, mu_a, mu_b, mu_c, acc2, sc, sh, locs = carry
            i1, _, i2, ir, i3 = locs
            v1, v2, v3 = inst(i1), inst(i2), inst(i3)
            nq = INST // SLAB
            new_acc1 = _tree_sum([jnp.sum(ld(v1, q), axis=0) for q in range(nq)])
            if start_next is not None:
                start_next()
            parts = []
            for q in range(nq):
                d = ld(v2, q) - mu_a
                parts.append(jnp.sum(d * d, axis=0))
            new_acc2 = _tree_sum(parts)
            new_mu = _full_sum_bcast(acc1) * inv_n
            ch = (base * per_super + ir) & (C - 1)
            var = _full_sum_bcast(acc2) * inv_n
            new_sc = jax.lax.rsqrt(var + EPS) * g_s[ch].astype(f32)
            new_sh = jnp.full((8, LANES), b_s[ch].astype(f32), f32)
            if normalise:
                for q in range(nq):
                    y = (ld(v3, q) - mu_c) * sc + sh
                    v3[pl.ds(SLAB * q, SLAB), :] = (
                        y.reshape(SLAB, LANES).astype(buf.dtype))
            new_locs = (loc(k + 1 - LAG),) + locs[:-1]
            return (new_acc1, new_mu, mu_a, mu_b, new_acc2, new_sc, new_sh, new_locs)

        first_reads(0)
        cg = pltpu.make_async_copy(g_hbm, g_s, wsem.at[0])
        cb = pltpu.make_async_copy(b_hbm, b_s, wsem.at[1])
        cg.start()
        cb.start()
        cg.wait()
        cb.wait()

        def group(gi, carry0):
            base = gi * GS

            def step_dma_only(k, c):
                read_wait(base, k)
                read_start(base, k + DEPTH, "regular")
                return c

            def step_fill(k, carry):
                read_wait(base, k)
                return stages(base, k, carry,
                              lambda: read_start(base, k + DEPTH, "regular"),
                              normalise=False)

            def step_main(k, carry):
                read_wait(base, k)
                return stages(base, k, carry, lambda: read_start(base, k + DEPTH))

            def step_tail(k, carry):
                @pl.when(k < M)
                def _():
                    read_wait(base, k)

                @pl.when(k == M - 1 - EARLY_AT)
                def _():
                    write_start(base, spans[0], 0, N_EARLY, wsem.at[0])

                @pl.when(k == M - 1)
                def _():
                    write_start(base, spans[0], N_EARLY, N_MID, wsem.at[0])

                return stages(base, k, carry)

            z = jnp.zeros((8, LANES), f32)
            carry = (z,) * 7 + ((jnp.int32(0),) * 5,)
            jax.lax.fori_loop(0, LAG, step_dma_only, 0)
            carry = jax.lax.fori_loop(LAG, LAG + 4, step_fill, carry)
            carry = jax.lax.fori_loop(LAG + 4, M - DEPTH, step_main, carry)
            jax.lax.fori_loop(M - DEPTH, M + LAG + 4, step_tail, carry)

            last = spans[-1]
            for span in spans:
                u0 = N_MID if span == spans[0] else 0
                u1 = NU - WUNROLL if span == last else NU
                write_loop(base, span, u0, u1, wsem.at[0])
            write_start(base, last, NU - WUNROLL, NU - 1, wsem.at[0])
            write_start(base, last, NU - 1, NU, wsem.at[1])
            for span in spans[:-1]:
                wr(base, span, (), wsem.at[0]).wait()
            wr(base, last, (pl.ds(0, NA - 1),), wsem.at[0]).wait()
            wr(base, last, (NA - 1, 0), wsem.at[0]).wait()
            wr(base, last, (NA - 1, 1, pl.ds(0, ROW - PIECE)), wsem.at[0]).wait()

            @pl.when(gi + 1 < ngroups)
            def _():
                first_reads(base + GS)

            wr(base, last, (NA - 1, 1, pl.ds(ROW - PIECE, PIECE)), wsem.at[1]).wait()
            return carry0

        jax.lax.fori_loop(0, ngroups, group, 0)

    view = (NS, NA, NH, ROW, LANES)
    xt = x.transpose(0, 1, 3, 2).reshape(n_inst, W // 8, 8, H // LANES, LANES)
    xt = xt.transpose(0, 1, 3, 2, 4).reshape(view)
    y = pl.pallas_call(
        kernel,
        in_specs=[pl.BlockSpec(memory_space=pl.ANY)] * 3,
        out_specs=pl.BlockSpec(memory_space=pl.ANY),
        out_shape=jax.ShapeDtypeStruct(view, x.dtype),
        scratch_shapes=[
            pltpu.VMEM((GS,) + view[1:], x.dtype),
            pltpu.SMEM((C,), g.dtype),
            pltpu.SMEM((C,), b.dtype),
            pltpu.SemaphoreType.DMA((DEPTH,)),
            pltpu.SemaphoreType.DMA((2,)),
        ],
        compiler_params=pltpu.CompilerParams(
            vmem_limit_bytes=min(GS * 8 + 4, 128) * 1024 * 1024,
            disable_bounds_checks=True),
    )(xt, g, b)
    y = y.reshape(n_inst, W // 8, H // LANES, 8, LANES).transpose(0, 1, 3, 2, 4)
    return y.reshape(B, C, W, H).transpose(0, 1, 3, 2)
```

```python
import jax
import jax.numpy as jnp
import jax.experimental.pallas as pl
import jax.experimental.pallas.tpu as pltpu

EPS = 1e-5
LANES = 128
INST = 512
NJ = 8
NA, NH = 4, 2
ROW = NJ * INST
PIECE = 128
NP = ROW // PIECE
SLAB = 64
HALF = 256
GS = 16
SPANS = (8, 8)
DEPTH = 8
SHIFT = 104
LO_ROW = (0, 1)
HI_ROW = (3, 0)
LAG = 9
EARLY_AT = 4
N_EARLY = 48
N_TAIL = 1
WUNROLL = 8


def _tree_sum(xs):
    xs = list(xs)
    while len(xs) > 1:
        nxt = [xs[i] + xs[i + 1] for i in range(0, len(xs) - 1, 2)]
        if len(xs) % 2:
            nxt.append(xs[-1])
        xs = nxt
    return xs[0]


def _full_sum_bcast(acc):
    s = jnp.sum(jnp.sum(acc, axis=0, keepdims=True), axis=1, keepdims=True)
    return jnp.broadcast_to(s, acc.shape)


@jax.jit
def pallas_standalone__instancenorm__prompt_kernel(
    x: jax.Array,
    g: jax.Array,
    b: jax.Array,
):
    B, C, H, W = x.shape
    n_inst = B * C
    per_super = NA * NH * NJ
    assert H * W == INST * LANES and W % 8 == 0 and H % LANES == 0
    assert C & (C - 1) == 0 and n_inst % (GS * per_super) == 0
    NS = n_inst // per_super
    ngroups = NS // GS
    M = GS * per_super
    assert sum(SPANS) == GS and len(SPANS) >= 2 and N_EARLY % WUNROLL == 0
    spans = [(sum(SPANS[:i]), n) for i, n in enumerate(SPANS)]
    NU = NA * NH * NP
    inv_n = 1.0 / (H * W)
    f32 = jnp.float32

    def kernel(x_hbm, g_hbm, b_hbm, o_hbm, buf, g_s, b_s, rsem, wsem):
        def rd(base, k, rows, off, size):
            s, h = k >> 6, k & 1
            return pltpu.make_async_copy(
                x_hbm.at[base + s, rows, h, pl.ds(off, size)],
                buf.at[s, rows, h, pl.ds(off, size)],
                rsem.at[k & (DEPTH - 1)])

        def read_start(base, k, kind=None):
            p = (k >> 1) & (NP - 1)
            h = k & 1

            def regular():
                off = pl.multiple_of(p * PIECE + (SHIFT - PIECE), 8)
                lo = LO_ROW[0] + h * (LO_ROW[1] - LO_ROW[0])
                hi = HI_ROW[0] + h * (HI_ROW[1] - HI_ROW[0])
                rd(base, k, pl.ds(lo, NA - 1), off, PIECE).start(priority=1)
                rd(base, k, pl.ds(hi, 1), off, PIECE).start(priority=0)

            def ends():
                rows = pl.ds(0, NA)
                rd(base, k, rows, 0, SHIFT).start(priority=1)
                rd(base, k, rows, ROW - PIECE + SHIFT, PIECE - SHIFT).start(priority=0)

            if kind == "static":
                (ends if p == 0 else regular)()
            elif kind == "regular":
                regular()
            else:
                pl.when(p != 0)(regular)
                pl.when(p == 0)(ends)

        def read_wait(base, k):
            rd(base, k, pl.ds(0, NA), 0, PIECE).wait()

        def first_reads(base):
            for k in range(DEPTH):
                read_start(base, k, "static")

        def wr(base, span, idx, sem):
            s0, n = span
            return pltpu.make_async_copy(
                buf.at[(pl.ds(s0, n),) + idx],
                o_hbm.at[(pl.ds(base + s0, n),) + idx], sem)

        def write_start(base, span, u0, u1, sem):
            for u in range(u0, u1):
                r = u // NP
                idx = (r // NH, r % NH, pl.ds((u % NP) * PIECE, PIECE))
                wr(base, span, idx, sem).start()

        def write_loop(base, span, u0, u1, sem):
            def body(t, c):
                u = t * WUNROLL
                r = u >> 5
                off = pl.multiple_of((u & (NP - 1)) * PIECE, PIECE * WUNROLL)
                for i in range(WUNROLL):
                    idx = (r >> 1, r & 1, pl.ds(off + i * PIECE, PIECE))
                    wr(base, span, idx, sem).start()
                return c

            jax.lax.fori_loop(u0 // WUNROLL, u1 // WUNROLL, body, 0)

        def loc(m):
            m = jnp.minimum(m, M - 1)
            return (m & ~63) + ((m & 7) << 3) + ((m >> 3) & 7)

        def inst(i):
            start = pl.multiple_of((i & 7) * INST, INST)
            return buf.at[i >> 6, (i >> 4) & 3, (i >> 3) & 1, pl.ds(start, INST)]

        def to_f32(v):
            return v.astype(f32).reshape(v.shape[0] // 8, 8, LANES)

        def stages(base, k, carry, start_next=None, normalise=True):
            acc1, mu_a, mu_b, mu_c, acc2, sc, sh, locs = carry
            i1, _, i2, ir, i3 = locs
            v1, v2, v3 = inst(i1), inst(i2), inst(i3)
            x1 = v1[...]
            new_acc1 = _tree_sum([jnp.sum(to_f32(x1[q:q + SLAB]), axis=0)
                                  for q in range(0, INST, SLAB)])
            if start_next is not None:
                start_next()
            x2 = v2[...]
            parts = []
            for q in range(0, INST, SLAB):
                d = to_f32(x2[q:q + SLAB]) - mu_a
                parts.append(jnp.sum(d * d, axis=0))
            new_acc2 = _tree_sum(parts)
            new_mu = _full_sum_bcast(acc1) * inv_n
            ch = (base * per_super + ir) & (C - 1)
            var = _full_sum_bcast(acc2) * inv_n
            new_sc = jax.lax.rsqrt(var + EPS) * g_s[ch].astype(f32)
            new_sh = jnp.full((8, LANES), b_s[ch].astype(f32), f32)
            if normalise:
                for q in range(0, INST, HALF):
                    y = (to_f32(v3[pl.ds(q, HALF), :]) - mu_c) * sc + sh
                    v3[pl.ds(q, HALF), :] = y.reshape(HALF, LANES).astype(buf.dtype)
            new_locs = (loc(k + 1 - LAG),) + locs[:-1]
            return (new_acc1, new_mu, mu_a, mu_b, new_acc2, new_sc, new_sh, new_locs)

        first_reads(0)
        cg = pltpu.make_async_copy(g_hbm, g_s, wsem.at[0])
        cb = pltpu.make_async_copy(b_hbm, b_s, wsem.at[1])
        cg.start()
        cb.start()
        cg.wait()
        cb.wait()

        def group(gi, carry0):
            base = gi * GS

            def step_dma_only(k, c):
                read_wait(base, k)
                read_start(base, k + DEPTH, "regular")
                return c

            def step_fill(k, carry):
                read_wait(base, k)
                return stages(base, k, carry,
                              lambda: read_start(base, k + DEPTH, "regular"),
                              normalise=False)

            def step_main(k, carry):
                read_wait(base, k)
                return stages(base, k, carry, lambda: read_start(base, k + DEPTH))

            def step_tail(k, carry):
                @pl.when(k < M)
                def _():
                    read_wait(base, k)

                @pl.when(k == M - 1 - EARLY_AT)
                def _():
                    write_start(base, spans[0], 0, N_EARLY, wsem.at[0])

                return stages(base, k, carry)

            z = jnp.zeros((8, LANES), f32)
            carry = (z,) * 7 + ((jnp.int32(0),) * 5,)
            jax.lax.fori_loop(0, LAG, step_dma_only, 0)
            carry = jax.lax.fori_loop(LAG, LAG + 4, step_fill, carry)
            carry = jax.lax.fori_loop(LAG + 4, M - DEPTH, step_main, carry)
            jax.lax.fori_loop(M - DEPTH, M + LAG + 4, step_tail, carry)

            last = spans[-1]
            for span in spans:
                u0 = N_EARLY if span == spans[0] else 0
                u1 = NU - WUNROLL if span == last else NU
                write_loop(base, span, u0, u1, wsem.at[0])
            write_start(base, last, NU - WUNROLL, NU - N_TAIL, wsem.at[0])
            write_start(base, last, NU - N_TAIL, NU, wsem.at[1])
            cut = ROW - N_TAIL * PIECE
            for span in spans[:-1]:
                wr(base, span, (), wsem.at[0]).wait()
            wr(base, last, (pl.ds(0, NA - 1),), wsem.at[0]).wait()
            wr(base, last, (NA - 1, 0), wsem.at[0]).wait()
            wr(base, last, (NA - 1, 1, pl.ds(0, cut)), wsem.at[0]).wait()

            @pl.when(gi + 1 < ngroups)
            def _():
                first_reads(base + GS)

            wr(base, last, (NA - 1, 1, pl.ds(cut, ROW - cut)), wsem.at[1]).wait()
            return carry0

        jax.lax.fori_loop(0, ngroups, group, 0)

    view = (NS, NA, NH, ROW, LANES)
    xt = x.transpose(0, 1, 3, 2).reshape(n_inst, W // 8, 8, H // LANES, LANES)
    xt = xt.transpose(0, 1, 3, 2, 4).reshape(view)
    y = pl.pallas_call(
        kernel,
        in_specs=[pl.BlockSpec(memory_space=pl.ANY)] * 3,
        out_specs=pl.BlockSpec(memory_space=pl.ANY),
        out_shape=jax.ShapeDtypeStruct(view, x.dtype),
        scratch_shapes=[
            pltpu.VMEM((GS,) + view[1:], x.dtype),
            pltpu.SMEM((C,), g.dtype),
            pltpu.SMEM((C,), b.dtype),
            pltpu.SemaphoreType.DMA((DEPTH,)),
            pltpu.SemaphoreType.DMA((2,)),
        ],
        compiler_params=pltpu.CompilerParams(
            vmem_limit_bytes=min(GS * 8 + 4, 128) * 1024 * 1024,
            disable_bounds_checks=True),
    )(xt, g, b)
    y = y.reshape(n_inst, W // 8, H // LANES, 8, LANES).transpose(0, 1, 3, 2, 4)
    return y.reshape(B, C, W, H).transpose(0, 1, 3, 2)
```

```python
import jax
import jax.numpy as jnp
import jax.experimental.pallas as pl
import jax.experimental.pallas.tpu as pltpu

EPS = 1e-5
LANES = 128
INST = 512
NJ = 8
NA, NH = 4, 2
ROW = NJ * INST
SLAB = 64
HALF = 256
GS = 16

RPIECE = 256
SHIFT = 104
DEPTH = 8
NSEM = 8
LO_ROW = (0, 1)
HI_ROW = (3, 0)
LAG = 11

PIECE = 128
NP = ROW // PIECE
SPANS = (8, 8)
EARLY_AT = 5
N_EARLY = 24
WUNROLL = 8


def _tree_sum(xs):
    xs = list(xs)
    while len(xs) > 1:
        nxt = [xs[i] + xs[i + 1] for i in range(0, len(xs) - 1, 2)]
        if len(xs) % 2:
            nxt.append(xs[-1])
        xs = nxt
    return xs[0]


def _full_sum_bcast(acc):
    s = jnp.sum(jnp.sum(acc, axis=0, keepdims=True), axis=1, keepdims=True)
    return jnp.broadcast_to(s, acc.shape)


@jax.jit
def pallas_standalone__instancenorm__prompt_kernel(
    x: jax.Array,
    g: jax.Array,
    b: jax.Array,
):
    B, C, H, W = x.shape
    n_inst = B * C
    per_super = NA * NH * NJ
    assert H * W == INST * LANES and W % 8 == 0 and H % LANES == 0
    assert C & (C - 1) == 0 and n_inst % (GS * per_super) == 0
    NS = n_inst // per_super
    ngroups = NS // GS
    M = GS * per_super
    assert DEPTH % 2 == 0 and DEPTH // 2 < NSEM and 0 < SHIFT < RPIECE
    assert sum(SPANS) == GS and len(SPANS) >= 2 and N_EARLY % WUNROLL == 0
    spans = [(sum(SPANS[:i]), n) for i, n in enumerate(SPANS)]
    NU = NA * NH * NP
    inv_n = 1.0 / (H * W)
    f32 = jnp.float32

    def kernel(x_hbm, g_hbm, b_hbm, o_hbm, buf, g_s, b_s, rsem, wsem):
        def rd(base, k, rows, off, size):
            s, h = k >> 6, (k >> 1) & 1
            return pltpu.make_async_copy(
                x_hbm.at[base + s, rows, h, pl.ds(off, size)],
                buf.at[s, rows, h, pl.ds(off, size)],
                rsem.at[(k >> 1) & (NSEM - 1)])

        def read_start(base, k, part, kind=None):
            p = (k >> 2) & (ROW // RPIECE - 1)
            h = (k >> 1) & 1
            e = k & 1
            lo = pl.ds(LO_ROW[0] + h * (LO_ROW[1] - LO_ROW[0]), NA - 1)
            hi = pl.ds(HI_ROW[0] + h * (HI_ROW[1] - HI_ROW[0]), 1)
            tail = ROW - RPIECE + SHIFT

            def when(cond):
                if kind == "static":
                    return (lambda f: f()) if cond else (lambda f: None)
                return pl.when(cond)

            def regular():
                off = pl.multiple_of(p * RPIECE + (SHIFT - RPIECE), 8)
                if part == 0:
                    @when(e == 0)
                    def _():
                        rd(base, k, lo, off, RPIECE).start(priority=1)

                quarter = RPIECE // 4
                off_hi = pl.multiple_of(off + e * (2 * quarter) + part * quarter, 8)
                rd(base, k, hi, off_hi, quarter).start(priority=0)

            def ends():
                @when(e == 0)
                def _():
                    rd(base, k, lo, 0, SHIFT).start(priority=1)
                    rd(base, k, lo, tail, ROW - tail).start(priority=1)
                    rd(base, k, hi, 0, SHIFT).start(priority=0)

                @when(e == 1)
                def _():
                    rd(base, k, hi, tail, ROW - tail).start(priority=0)

            if kind == "regular":
                regular()
            else:
                when(p != 0)(regular)
                if part == 1:
                    when(p == 0)(ends)

        def read_wait(base, k):
            rd(base, k, pl.ds(0, NA), 0, RPIECE // 2).wait()

        def first_reads(base):
            for k in range(DEPTH):
                read_start(base, k, 0, "static")
                read_start(base, k, 1, "static")

        def wr(base, span, idx, sem):
            s0, n = span
            return pltpu.make_async_copy(
                buf.at[(pl.ds(s0, n),) + idx],
                o_hbm.at[(pl.ds(base + s0, n),) + idx], sem)

        def write_start(base, span, u0, u1, sem):
            for u in range(u0, u1):
                r = u // NP
                idx = (r // NH, r % NH, pl.ds((u % NP) * PIECE, PIECE))
                wr(base, span, idx, sem).start()

        def write_loop(base, span, u0, u1, sem):
            def body(t, c):
                u = t * WUNROLL
                r = u >> 5
                off = pl.multiple_of((u & (NP - 1)) * PIECE, PIECE * WUNROLL)
                for i in range(WUNROLL):
                    idx = (r >> 1, r & 1, pl.ds(off + i * PIECE, PIECE))
                    wr(base, span, idx, sem).start()
                return c

            jax.lax.fori_loop(u0 // WUNROLL, u1 // WUNROLL, body, 0)

        def loc(m):
            m = jnp.minimum(m, M - 1)
            return (m & ~63) + ((m & 7) << 3) + ((m >> 3) & 7)

        def inst(i):
            start = pl.multiple_of((i & 7) * INST, INST)
            return buf.at[i >> 6, (i >> 4) & 3, (i >> 3) & 1, pl.ds(start, INST)]

        def to_f32(v):
            return v.astype(f32).reshape(v.shape[0] // 8, 8, LANES)

        def stages(base, k, carry, start_next=None, normalise=True):
            acc1, mu_a, mu_b, mu_c, acc2, sc, sh, locs = carry
            i1, _, i2, ir, i3 = locs
            v1, v2, v3 = inst(i1), inst(i2), inst(i3)
            x1 = v1[...]
            new_acc1 = _tree_sum([jnp.sum(to_f32(x1[q:q + SLAB]), axis=0)
                                  for q in range(0, INST, SLAB)])
            if start_next is not None:
                start_next(0)
            x2 = v2[...]
            parts = []
            for q in range(0, INST, SLAB):
                d = to_f32(x2[q:q + SLAB]) - mu_a
                parts.append(jnp.sum(d * d, axis=0))
            new_acc2 = _tree_sum(parts)
            if start_next is not None:
                start_next(1)
            new_mu = _full_sum_bcast(acc1) * inv_n
            ch = (base * per_super + ir) & (C - 1)
            var = _full_sum_bcast(acc2) * inv_n
            new_sc = jax.lax.rsqrt(var + EPS) * g_s[ch].astype(f32)
            new_sh = jnp.full((8, LANES), b_s[ch].astype(f32), f32)
            if normalise:
                for q in range(0, INST, HALF):
                    y = (to_f32(v3[pl.ds(q, HALF), :]) - mu_c) * sc + sh
                    v3[pl.ds(q, HALF), :] = y.reshape(HALF, LANES).astype(buf.dtype)
            new_locs = (loc(k + 1 - LAG),) + locs[:-1]
            return (new_acc1, new_mu, mu_a, mu_b, new_acc2, new_sc, new_sh, new_locs)

        first_reads(0)
        cg = pltpu.make_async_copy(g_hbm, g_s, wsem.at[0])
        cb = pltpu.make_async_copy(b_hbm, b_s, wsem.at[1])
        cg.start()
        cb.start()
        cg.wait()
        cb.wait()

        def group(gi, carry0):
            base = gi * GS

            def step_dma_only(k, c):
                read_wait(base, k)
                read_start(base, k + DEPTH, 0, "regular")
                read_start(base, k + DEPTH, 1, "regular")
                return c

            def step_fill(k, carry):
                read_wait(base, k)
                return stages(base, k, carry,
                              lambda part: read_start(base, k + DEPTH, part, "regular"),
                              normalise=False)

            def step_main(k, carry):
                read_wait(base, k)
                return stages(base, k, carry,
                              lambda part: read_start(base, k + DEPTH, part))

            def step_tail(k, carry):
                @pl.when(k < M)
                def _():
                    read_wait(base, k)

                @pl.when(k == M - 1 - EARLY_AT)
                def _():
                    write_start(base, spans[0], 0, N_EARLY, wsem.at[0])

                return stages(base, k, carry)

            z = jnp.zeros((8, LANES), f32)
            carry = (z,) * 7 + ((jnp.int32(0),) * 5,)
            jax.lax.fori_loop(0, LAG, step_dma_only, 0)
            carry = jax.lax.fori_loop(LAG, LAG + 4, step_fill, carry)
            carry = jax.lax.fori_loop(LAG + 4, M - DEPTH, step_main, carry)
            jax.lax.fori_loop(M - DEPTH, M + LAG + 4, step_tail, carry)

            last = spans[-1]
            for span in spans:
                u0 = N_EARLY if span == spans[0] else 0
                u1 = NU - WUNROLL if span == last else NU
                write_loop(base, span, u0, u1, wsem.at[0])
            write_start(base, last, NU - WUNROLL, NU - 1, wsem.at[0])
            write_start(base, last, NU - 1, NU, wsem.at[1])
            for span in spans[:-1]:
                wr(base, span, (), wsem.at[0]).wait()
            wr(base, last, (pl.ds(0, NA - 1),), wsem.at[0]).wait()
            wr(base, last, (NA - 1, 0), wsem.at[0]).wait()
            wr(base, last, (NA - 1, 1, pl.ds(0, ROW - PIECE)), wsem.at[0]).wait()

            @pl.when(gi + 1 < ngroups)
            def _():
                first_reads(base + GS)

            wr(base, last, (NA - 1, 1, pl.ds(ROW - PIECE, PIECE)), wsem.at[1]).wait()
            return carry0

        jax.lax.fori_loop(0, ngroups, group, 0)

    view = (NS, NA, NH, ROW, LANES)
    xt = x.transpose(0, 1, 3, 2).reshape(n_inst, W // 8, 8, H // LANES, LANES)
    xt = xt.transpose(0, 1, 3, 2, 4).reshape(view)
    y = pl.pallas_call(
        kernel,
        in_specs=[pl.BlockSpec(memory_space=pl.ANY)] * 3,
        out_specs=pl.BlockSpec(memory_space=pl.ANY),
        out_shape=jax.ShapeDtypeStruct(view, x.dtype),
        scratch_shapes=[
            pltpu.VMEM((GS,) + view[1:], x.dtype),
            pltpu.SMEM((C,), g.dtype),
            pltpu.SMEM((C,), b.dtype),
            pltpu.SemaphoreType.DMA((NSEM,)),
            pltpu.SemaphoreType.DMA((2,)),
        ],
        compiler_params=pltpu.CompilerParams(
            vmem_limit_bytes=min(GS * 8 + 4, 128) * 1024 * 1024,
            disable_bounds_checks=True),
    )(xt, g, b)
    y = y.reshape(n_inst, W // 8, H // LANES, 8, LANES).transpose(0, 1, 3, 2, 4)
    return y.reshape(B, C, W, H).transpose(0, 1, 3, 2)
```

```python
import jax
import jax.numpy as jnp
import jax.experimental.pallas as pl
import jax.experimental.pallas.tpu as pltpu

EPS = 1e-5
LANES = 128
INST = 512
NJ = 8
NA, NH = 4, 2
ROW = NJ * INST
SLAB = 64
HALF = 256
GS = 16

RPIECE = 256
SHIFT = 104
DEPTH = 8
NSEM = 8
LO_ROW = (0, 1)
HI_ROW = (3, 0)
LAG = 12

PIECE = 128
NP = ROW // PIECE
SPANS = (8, 8)
EARLY_AT = 5
N_EARLY = 48
WUNROLL = 8


def _tree_sum(xs):
    xs = list(xs)
    while len(xs) > 1:
        nxt = [xs[i] + xs[i + 1] for i in range(0, len(xs) - 1, 2)]
        if len(xs) % 2:
            nxt.append(xs[-1])
        xs = nxt
    return xs[0]


def _full_sum_bcast(acc):
    s = jnp.sum(jnp.sum(acc, axis=0, keepdims=True), axis=1, keepdims=True)
    return jnp.broadcast_to(s, acc.shape)


@jax.jit
def pallas_standalone__instancenorm__prompt_kernel(
    x: jax.Array,
    g: jax.Array,
    b: jax.Array,
):
    B, C, H, W = x.shape
    n_inst = B * C
    per_super = NA * NH * NJ
    assert H * W == INST * LANES and W % 8 == 0 and H % LANES == 0
    assert C & (C - 1) == 0 and n_inst % (GS * per_super) == 0
    NS = n_inst // per_super
    ngroups = NS // GS
    M = GS * per_super
    assert DEPTH % 2 == 0 and DEPTH // 2 < NSEM and 0 < SHIFT < RPIECE
    assert sum(SPANS) == GS and len(SPANS) >= 2 and N_EARLY % WUNROLL == 0
    spans = [(sum(SPANS[:i]), n) for i, n in enumerate(SPANS)]
    NU = NA * NH * NP
    FILLED = LAG + 4
    assert FILLED % 2 == 0
    inv_n = 1.0 / (H * W)
    f32 = jnp.float32

    def kernel(x_hbm, g_hbm, b_hbm, o_hbm, buf, g_s, b_s, lsem, hsem, wsem):
        def read_ops(base, k, kind, e=None):
            s, h = k >> 6, (k >> 1) & 1
            e = k & 1 if e is None else e
            p = (k >> 2) & (ROW // RPIECE - 1)
            slot = (k >> 1) & (NSEM - 1)
            tail = ROW - RPIECE + SHIFT

            def desc(rows, sem, off, size):
                return pltpu.make_async_copy(
                    x_hbm.at[base + s, rows, h, pl.ds(off, size)],
                    buf.at[s, rows, h, pl.ds(off, size)], sem.at[slot])

            def lo(off, size):
                r0 = LO_ROW[0] + h * (LO_ROW[1] - LO_ROW[0])
                return desc(pl.ds(r0, NA - 1), lsem, off, size)

            def hi(off, size):
                r0 = HI_ROW[0] + h * (HI_ROW[1] - HI_ROW[0])
                return desc(pl.ds(r0, 1), hsem, off, size)

            def when(cond):
                if isinstance(cond, bool):
                    return (lambda f: f()) if cond else (lambda f: None)
                return pl.when(cond)

            def select(regular, ends):
                def reg():
                    regular(pl.multiple_of(p * RPIECE + (SHIFT - RPIECE), 8))

                if kind == "regular":
                    reg()
                else:
                    when(p != 0)(reg)
                    if ends is not None:
                        when(p == 0)(lambda: ends((0, SHIFT), (tail, ROW - tail)))

            return e, lo, hi, when, select

        def read_start(base, k, part, kind=None, e=None):
            e, lo, hi, when, select = read_ops(base, k, kind, e)

            def regular(off):
                if part == 0:
                    when(e == 0)(lambda: lo(off, RPIECE).start(priority=1))
                quarter = RPIECE // 4
                off_hi = pl.multiple_of(off + e * (2 * quarter) + part * quarter, 8)
                hi(off_hi, quarter).start(priority=0)

            def ends(head, tail):
                @when(e == 0)
                def _():
                    lo(*head).start(priority=1)
                    lo(*tail).start(priority=1)
                    hi(*head).start(priority=0)

                @when(e == 1)
                def _():
                    hi(*tail).start(priority=0)

            select(regular, ends if part == 1 else None)

        def read_wait(base, k, kind=None, e=None):
            e, lo, hi, when, select = read_ops(base, k, kind, e)
            for parity, rows in ((0, hi), (1, lo)):
                def regular(off):
                    rows(off, RPIECE).wait()

                def ends(head, tail):
                    rows(*head).wait()
                    rows(*tail).wait()

                when(e == parity)(lambda: select(regular, ends))

        def first_reads(base):
            for k in range(DEPTH):
                read_start(base, k, 0, "static")
                read_start(base, k, 1, "static")

        def wr(base, span, idx, sem):
            s0, n = span
            return pltpu.make_async_copy(
                buf.at[(pl.ds(s0, n),) + idx],
                o_hbm.at[(pl.ds(base + s0, n),) + idx], sem)

        def write_start(base, span, u0, u1, sem):
            for u in range(u0, u1):
                r = u // NP
                idx = (r // NH, r % NH, pl.ds((u % NP) * PIECE, PIECE))
                wr(base, span, idx, sem).start()

        def write_loop(base, span, u0, u1, sem_of_row):
            def body(t, c):
                u = t * WUNROLL
                r = u >> 5
                sem = sem_of_row(r)
                off = pl.multiple_of((u & (NP - 1)) * PIECE, PIECE * WUNROLL)
                for i in range(WUNROLL):
                    idx = (r >> 1, r & 1, pl.ds(off + i * PIECE, PIECE))
                    wr(base, span, idx, sem).start()
                return c

            jax.lax.fori_loop(u0 // WUNROLL, u1 // WUNROLL, body, 0)

        def loc(m):
            m = jnp.minimum(m, M - 1)
            return (m & ~63) + ((m & 7) << 3) + ((m >> 3) & 7)

        def inst(i):
            start = pl.multiple_of((i & 7) * INST, INST)
            return buf.at[i >> 6, (i >> 4) & 3, (i >> 3) & 1, pl.ds(start, INST)]

        def to_f32(v):
            return v.astype(f32).reshape(v.shape[0] // 8, 8, LANES)

        def stages(base, k, carry, start_next=None, normalise=True):
            acc1, mu_a, mu_b, mu_c, acc2, sc, sh, locs = carry
            i1, _, i2, ir, i3 = locs
            v1, v2, v3 = inst(i1), inst(i2), inst(i3)
            x1 = v1[...]
            new_acc1 = _tree_sum([jnp.sum(to_f32(x1[q:q + SLAB]), axis=0)
                                  for q in range(0, INST, SLAB)])
            if start_next is not None:
                start_next(0)
            x2 = v2[...]
            parts = []
            for q in range(0, INST, SLAB):
                d = to_f32(x2[q:q + SLAB]) - mu_a
                parts.append(jnp.sum(d * d, axis=0))
            new_acc2 = _tree_sum(parts)
            if start_next is not None:
                start_next(1)
            new_mu = _full_sum_bcast(acc1) * inv_n
            ch = (base * per_super + ir) & (C - 1)
            var = _full_sum_bcast(acc2) * inv_n
            new_sc = jax.lax.rsqrt(var + EPS) * g_s[ch].astype(f32)
            new_sh = jnp.full((8, LANES), b_s[ch].astype(f32), f32)
            if normalise:
                for q in range(0, INST, HALF):
                    y = (to_f32(v3[pl.ds(q, HALF), :]) - mu_c) * sc + sh
                    v3[pl.ds(q, HALF), :] = y.reshape(HALF, LANES).astype(buf.dtype)
            new_locs = (loc(k + 1 - LAG),) + locs[:-1]
            return (new_acc1, new_mu, mu_a, mu_b, new_acc2, new_sc, new_sh, new_locs)

        first_reads(0)
        cg = pltpu.make_async_copy(g_hbm, g_s, wsem.at[0])
        cb = pltpu.make_async_copy(b_hbm, b_s, wsem.at[1])
        cg.start()
        cb.start()
        cg.wait()
        cb.wait()

        def group(gi, carry0):
            base = gi * GS

            def step_dma_only(k, c):
                read_wait(base, k)
                read_start(base, k + DEPTH, 0, "regular")
                read_start(base, k + DEPTH, 1, "regular")
                return c

            def step_fill(k, carry):
                read_wait(base, k, "regular")
                return stages(base, k, carry,
                              lambda part: read_start(base, k + DEPTH, part, "regular"),
                              normalise=False)

            def step_main(k, carry):
                read_wait(base, k)
                return stages(base, k, carry,
                              lambda part: read_start(base, k + DEPTH, part))

            def unit_lean(u, carry):
                for e in range(2):
                    k = 2 * u + e
                    read_wait(base, k, "regular", e)
                    carry = stages(base, k, carry, lambda part: read_start(
                        base, k + DEPTH, part, "regular", e))
                return carry

            def super_row(s, carry):
                k0 = jnp.maximum(s * per_super + 4, FILLED)
                k1 = (s + 1) * per_super - DEPTH
                k2 = jnp.minimum((s + 1) * per_super + 4, M - DEPTH)
                carry = jax.lax.fori_loop(k0 >> 1, k1 >> 1, unit_lean, carry)
                return jax.lax.fori_loop(k1, k2, step_main, carry)

            def step_tail(k, carry):
                @pl.when(k < M)
                def _():
                    read_wait(base, k, "regular")

                @pl.when(k == M - 1 - EARLY_AT)
                def _():
                    write_start(base, spans[0], 0, N_EARLY, wsem.at[0])

                return stages(base, k, carry)

            z = jnp.zeros((8, LANES), f32)
            carry = (z,) * 7 + ((jnp.int32(0),) * 5,)
            jax.lax.fori_loop(0, LAG, step_dma_only, 0)
            carry = jax.lax.fori_loop(LAG, LAG + 4, step_fill, carry)
            carry = jax.lax.fori_loop(0, GS, super_row, carry)
            jax.lax.fori_loop(M - DEPTH, M + LAG + 4, step_tail, carry)

            nl = len(spans) - 1
            last = spans[nl]
            for i, span in enumerate(spans[:nl]):
                write_loop(base, span, N_EARLY if i == 0 else 0, NU,
                           lambda r, i=i: wsem.at[i])
            write_loop(base, last, 0, NU - WUNROLL,
                       lambda r: wsem.at[nl + jnp.maximum(r - (NA * NH - 3), 0)])
            write_start(base, last, NU - WUNROLL, NU - 1, wsem.at[nl + 2])
            write_start(base, last, NU - 1, NU, wsem.at[nl + 3])
            for i, span in enumerate(spans[:nl]):
                wr(base, span, (), wsem.at[i]).wait()
            wr(base, last, (pl.ds(0, NA - 1),), wsem.at[nl]).wait()
            wr(base, last, (NA - 1, 0), wsem.at[nl + 1]).wait()
            wr(base, last, (NA - 1, 1, pl.ds(0, ROW - PIECE)), wsem.at[nl + 2]).wait()

            @pl.when(gi + 1 < ngroups)
            def _():
                first_reads(base + GS)

            wr(base, last, (NA - 1, 1, pl.ds(ROW - PIECE, PIECE)), wsem.at[nl + 3]).wait()
            return carry0

        jax.lax.fori_loop(0, ngroups, group, 0)

    view = (NS, NA, NH, ROW, LANES)
    xt = x.transpose(0, 1, 3, 2).reshape(n_inst, W // 8, 8, H // LANES, LANES)
    xt = xt.transpose(0, 1, 3, 2, 4).reshape(view)
    y = pl.pallas_call(
        kernel,
        in_specs=[pl.BlockSpec(memory_space=pl.ANY)] * 3,
        out_specs=pl.BlockSpec(memory_space=pl.ANY),
        out_shape=jax.ShapeDtypeStruct(view, x.dtype),
        scratch_shapes=[
            pltpu.VMEM((GS,) + view[1:], x.dtype),
            pltpu.SMEM((C,), g.dtype),
            pltpu.SMEM((C,), b.dtype),
            pltpu.SemaphoreType.DMA((NSEM,)),
            pltpu.SemaphoreType.DMA((NSEM,)),
            pltpu.SemaphoreType.DMA((len(SPANS) + 3,)),
        ],
        compiler_params=pltpu.CompilerParams(
            vmem_limit_bytes=min(GS * 8 + 4, 128) * 1024 * 1024,
            disable_bounds_checks=True,
            disable_semaphore_checks=True),
    )(xt, g, b)
    y = y.reshape(n_inst, W // 8, H // LANES, 8, LANES).transpose(0, 1, 3, 2, 4)
    return y.reshape(B, C, W, H).transpose(0, 1, 3, 2)
```

```python
import jax
import jax.numpy as jnp
import jax.experimental.pallas as pl
import jax.experimental.pallas.tpu as pltpu

EPS = 1e-5
SUB, LANES = 8, 128
INST = 64
NJ = 8
NA, NH = 4, 2
ROW = NJ * INST
SLAB = 16
HALF = 32
GS = 16

RPIECE = 32
SHIFT = 13
DEPTH = 8
NSEM = 8
LO_ROW = (0, 1)
HI_ROW = (3, 0)
LAG = 12

PIECE = 16
NP = ROW // PIECE
SPANS = (8, 8)
EARLY_AT = 5
N_EARLY = 72
WUNROLL = 8


def _tree_sum(xs):
    xs = list(xs)
    while len(xs) > 1:
        nxt = [xs[i] + xs[i + 1] for i in range(0, len(xs) - 1, 2)]
        if len(xs) % 2:
            nxt.append(xs[-1])
        xs = nxt
    return xs[0]


def _full_sum_bcast(acc):
    s = jnp.sum(jnp.sum(acc, axis=0, keepdims=True), axis=1, keepdims=True)
    return jnp.broadcast_to(s, acc.shape)


@jax.jit
def pallas_standalone__instancenorm__prompt_kernel(
    x: jax.Array,
    g: jax.Array,
    b: jax.Array,
):
    B, C, H, W = x.shape
    n_inst = B * C
    per_super = NA * NH * NJ
    assert H * W == INST * SUB * LANES and W % SUB == 0 and H % LANES == 0
    assert C & (C - 1) == 0 and n_inst % (GS * per_super) == 0
    NS = n_inst // per_super
    ngroups = NS // GS
    M = GS * per_super
    assert DEPTH % 2 == 0 and DEPTH // 2 < NSEM and 0 < SHIFT < RPIECE
    assert sum(SPANS) == GS and len(SPANS) >= 2 and N_EARLY % WUNROLL == 0
    spans = [(sum(SPANS[:i]), n) for i, n in enumerate(SPANS)]
    NU = NA * NH * NP
    FILLED = LAG + 4
    assert FILLED % 2 == 0
    inv_n = 1.0 / (H * W)
    f32 = jnp.float32

    def kernel(x_hbm, g_hbm, b_hbm, o_hbm, buf, g_s, b_s, lsem, hsem, wsem):
        def read_ops(base, k, kind, e=None):
            s, h = k >> 6, (k >> 1) & 1
            e = k & 1 if e is None else e
            p = (k >> 2) & (ROW // RPIECE - 1)
            slot = (k >> 1) & (NSEM - 1)
            tail = ROW - RPIECE + SHIFT

            def desc(rows, sem, off, size):
                return pltpu.make_async_copy(
                    x_hbm.at[base + s, rows, h, pl.ds(off, size)],
                    buf.at[s, rows, h, pl.ds(off, size)], sem.at[slot])

            def lo(off, size):
                r0 = LO_ROW[0] + h * (LO_ROW[1] - LO_ROW[0])
                return desc(pl.ds(r0, NA - 1), lsem, off, size)

            def hi(off, size):
                r0 = HI_ROW[0] + h * (HI_ROW[1] - HI_ROW[0])
                return desc(pl.ds(r0, 1), hsem, off, size)

            def when(cond):
                if isinstance(cond, bool):
                    return (lambda f: f()) if cond else (lambda f: None)
                return pl.when(cond)

            def select(regular, ends):
                def reg():
                    regular(p * RPIECE + (SHIFT - RPIECE))

                if kind == "regular":
                    reg()
                else:
                    when(p != 0)(reg)
                    if ends is not None:
                        when(p == 0)(lambda: ends((0, SHIFT), (tail, ROW - tail)))

            return e, lo, hi, when, select

        def read_start(base, k, part, kind=None, e=None):
            e, lo, hi, when, select = read_ops(base, k, kind, e)

            def regular(off):
                if part == 0:
                    when(e == 0)(lambda: lo(off, RPIECE).start(priority=1))
                quarter = RPIECE // 4
                hi(off + (2 * e + part) * quarter, quarter).start(priority=0)

            def ends(head, tail):
                @when(e == 0)
                def _():
                    lo(*head).start(priority=1)
                    lo(*tail).start(priority=1)
                    hi(*head).start(priority=0)

                @when(e == 1)
                def _():
                    hi(*tail).start(priority=0)

            select(regular, ends if part == 1 else None)

        def read_wait(base, k, kind=None, e=None):
            e, lo, hi, when, select = read_ops(base, k, kind, e)
            for parity, rows in ((0, hi), (1, lo)):
                def regular(off):
                    rows(off, RPIECE).wait()

                def ends(head, tail):
                    rows(*head).wait()
                    rows(*tail).wait()

                when(e == parity)(lambda: select(regular, ends))

        def first_reads(base):
            for k in range(DEPTH):
                read_start(base, k, 0)
                read_start(base, k, 1)

        def wr(base, span, idx, sem):
            s0, n = span
            return pltpu.make_async_copy(
                buf.at[(pl.ds(s0, n),) + idx],
                o_hbm.at[(pl.ds(base + s0, n),) + idx], sem)

        def write_start(base, span, u0, u1, sem):
            for u in range(u0, u1):
                r = u // NP
                idx = (r // NH, r % NH, pl.ds((u % NP) * PIECE, PIECE))
                wr(base, span, idx, sem).start()

        def write_loop(base, span, u0, u1, sem_of_row):
            def body(t, c):
                u = t * WUNROLL
                r = u >> 5
                sem = sem_of_row(r)
                off = (u & (NP - 1)) * PIECE
                for i in range(WUNROLL):
                    idx = (r >> 1, r & 1, pl.ds(off + i * PIECE, PIECE))
                    wr(base, span, idx, sem).start()
                return c

            jax.lax.fori_loop(u0 // WUNROLL, u1 // WUNROLL, body, 0)

        def loc(m):
            m = jnp.minimum(m, M - 1)
            return (m & ~63) + ((m & 7) << 3) + ((m >> 3) & 7)

        def inst(i):
            return buf.at[i >> 6, (i >> 4) & 3, (i >> 3) & 1, pl.ds((i & 7) * INST, INST)]

        def stages(base, k, carry, start_next=None, normalise=True):
            acc1, mu_a, mu_b, mu_c, acc2, sc, locs = carry
            i1, _, i2, ir, i3 = locs
            v1, v2, v3 = inst(i1), inst(i2), inst(i3)
            x1 = v1[...]
            new_acc1 = _tree_sum([jnp.sum(x1[q:q + SLAB].astype(f32), axis=0)
                                  for q in range(0, INST, SLAB)])
            if start_next is not None:
                start_next(0)
            x2 = v2[...]
            parts = []
            for q in range(0, INST, SLAB):
                d = x2[q:q + SLAB].astype(f32) - mu_a
                parts.append(jnp.sum(d * d, axis=0))
            new_acc2 = _tree_sum(parts)
            if start_next is not None:
                start_next(1)
            new_mu = _full_sum_bcast(acc1) * inv_n
            ch = (base * per_super + ir) & (C - 1)
            var = _full_sum_bcast(acc2) * inv_n
            new_sc = jax.lax.rsqrt(var + EPS) * g_s[ch].astype(f32)
            if normalise:
                sh = b_s[(base * per_super + i3) & (C - 1)].astype(f32)
                for q in range(0, INST, HALF):
                    y = (v3[pl.ds(q, HALF)].astype(f32) - mu_c) * sc + sh
                    v3[pl.ds(q, HALF)] = y.astype(buf.dtype)
            new_locs = (loc(k + 1 - LAG),) + locs[:-1]
            return (new_acc1, new_mu, mu_a, mu_b, new_acc2, new_sc, new_locs)

        first_reads(0)
        cg = pltpu.make_async_copy(g_hbm, g_s, wsem.at[0])
        cb = pltpu.make_async_copy(b_hbm, b_s, wsem.at[1])
        cg.start()
        cb.start()
        cg.wait()
        cb.wait()

        def group(gi, carry0):
            base = gi * GS

            def step_dma_only(k, c):
                read_wait(base, k)
                read_start(base, k + DEPTH, 0, "regular")
                read_start(base, k + DEPTH, 1, "regular")
                return c

            def step_fill(k, carry):
                read_wait(base, k, "regular")
                return stages(base, k, carry,
                              lambda part: read_start(base, k + DEPTH, part, "regular"),
                              normalise=False)

            def step_main(k, carry):
                read_wait(base, k)
                return stages(base, k, carry,
                              lambda part: read_start(base, k + DEPTH, part))

            def unit_lean(u, carry):
                for e in range(2):
                    k = 2 * u + e
                    read_wait(base, k, "regular", e)
                    carry = stages(base, k, carry, lambda part: read_start(
                        base, k + DEPTH, part, "regular", e))
                return carry

            def super_row(s, carry):
                k0 = jnp.maximum(s * per_super + 4, FILLED)
                k1 = (s + 1) * per_super - DEPTH
                k2 = jnp.minimum((s + 1) * per_super + 4, M - DEPTH)
                carry = jax.lax.fori_loop(k0 >> 1, k1 >> 1, unit_lean, carry)
                return jax.lax.fori_loop(k1, k2, step_main, carry)

            def step_tail(k, carry):
                @pl.when(k < M)
                def _():
                    read_wait(base, k, "regular")

                @pl.when(k == M - 1 - EARLY_AT)
                def _():
                    write_start(base, spans[0], 0, N_EARLY, wsem.at[0])

                return stages(base, k, carry)

            z = jnp.zeros((SUB, LANES), f32)
            carry = (z,) * 6 + ((jnp.int32(0),) * 5,)
            jax.lax.fori_loop(0, LAG, step_dma_only, 0)
            carry = jax.lax.fori_loop(LAG, FILLED, step_fill, carry)
            carry = jax.lax.fori_loop(0, GS, super_row, carry)
            jax.lax.fori_loop(M - DEPTH, M + FILLED, step_tail, carry)

            nl = len(spans) - 1
            last = spans[nl]
            for i, span in enumerate(spans[:nl]):
                write_loop(base, span, N_EARLY if i == 0 else 0, NU,
                           lambda r, i=i: wsem.at[i])
            write_loop(base, last, 0, NU - WUNROLL,
                       lambda r: wsem.at[nl + jnp.maximum(r - (NA * NH - 3), 0)])
            write_start(base, last, NU - WUNROLL, NU - 1, wsem.at[nl + 2])
            write_start(base, last, NU - 1, NU, wsem.at[nl + 3])
            for i, span in enumerate(spans[:nl]):
                wr(base, span, (), wsem.at[i]).wait()
            wr(base, last, (pl.ds(0, NA - 1),), wsem.at[nl]).wait()
            wr(base, last, (NA - 1, 0), wsem.at[nl + 1]).wait()
            wr(base, last, (NA - 1, 1, pl.ds(0, ROW - PIECE)), wsem.at[nl + 2]).wait()

            @pl.when(gi + 1 < ngroups)
            def _():
                first_reads(base + GS)

            wr(base, last, (NA - 1, 1, pl.ds(ROW - PIECE, PIECE)), wsem.at[nl + 3]).wait()
            return carry0

        jax.lax.fori_loop(0, ngroups, group, 0)

    view = (NS, NA, NH, ROW, SUB, LANES)
    xt = x.transpose(0, 1, 3, 2).reshape(n_inst, W // SUB, SUB, H // LANES, LANES)
    xt = xt.transpose(0, 1, 3, 2, 4).reshape(view)
    y = pl.pallas_call(
        kernel,
        in_specs=[pl.BlockSpec(memory_space=pl.ANY)] * 3,
        out_specs=pl.BlockSpec(memory_space=pl.ANY),
        out_shape=jax.ShapeDtypeStruct(view, x.dtype),
        scratch_shapes=[
            pltpu.VMEM((GS,) + view[1:], x.dtype),
            pltpu.SMEM((C,), g.dtype),
            pltpu.SMEM((C,), b.dtype),
            pltpu.SemaphoreType.DMA((NSEM,)),
            pltpu.SemaphoreType.DMA((NSEM,)),
            pltpu.SemaphoreType.DMA((len(SPANS) + 3,)),
        ],
        compiler_params=pltpu.CompilerParams(
            vmem_limit_bytes=min(GS * 8 + 4, 128) * 1024 * 1024,
            disable_bounds_checks=True,
            disable_semaphore_checks=True),
    )(xt, g, b)
    y = y.reshape(n_inst, W // SUB, H // LANES, SUB, LANES).transpose(0, 1, 3, 2, 4)
    return y.reshape(B, C, W, H).transpose(0, 1, 3, 2)
```
